```python
import os as _os
_os.environ.setdefault("JAX_PLATFORMS", "cpu")
import jax
import jax.numpy as jnp

def _softmax(x, axis=-1):
    return jax.nn.softmax(x, axis=axis)
def _gelu(x):
    return jax.nn.gelu(x, approximate=True)
def _silu(x):
    return jax.nn.silu(x)
def _sigmoid(x):
    return jax.nn.sigmoid(x)
def _layernorm(x, axis=-1, eps=1e-5):
    m = jnp.mean(x, axis=axis, keepdims=True)
    v = jnp.var(x, axis=axis, keepdims=True)
    return (x - m) / jnp.sqrt(v + eps)
def _scatter_add(tgt, idx, src, axis=0):
    return tgt.at[idx].add(src)
def _segment_sum(src, seg, n):
    return jax.ops.segment_sum(src, seg, n)
class _Rng:
    def __init__(self, key):
        self._k = key
    def _next(self):
        self._k, sub = jax.random.split(self._k)
        return sub
    def normal(self, shape):
        return jax.random.normal(self._next(), shape, dtype=jnp.bfloat16)
    def randint(self, lo, hi, shape):
        return jax.random.randint(self._next(), shape, lo, hi, dtype=jnp.int32)
    def uniform(self, shape, lo=0.0, hi=1.0):
        return jax.random.uniform(self._next(), shape, jnp.bfloat16, lo, hi)
    def permutation(self, n):
        return jax.random.permutation(self._next(), n)


kernel_name = 'parallel_sum__sliding_local_dilated__glu_gated_geglu__prompt'

def setup_inputs():
    _rng = _Rng(jax.random.key(int.from_bytes(__import__("os").urandom(4), "little")))
    _w = (lambda a: (lambda t: t.astype(jnp.bfloat16) if jnp.issubdtype(t.dtype, jnp.floating) else t)(jnp.asarray(a)))
    def _A_setup():
        B, S, D = 1, 2048, 512
        return {
            "x": _w((lambda *s: _rng.normal(s) * 0.05)(B, S, D)),
            "wqkv": _w((lambda *s: _rng.normal(s) * 0.05)(D, 3 * D)),
            "wo": _w((lambda *s: _rng.normal(s) * 0.05)(D, D)),
        }
    _A_in = _A_setup()

    def _B_setup():
        B, S, Dm, Df = 1, 2048, 512, 1376
        return {
            "x": _w((lambda *s: _rng.normal(s) * 0.05)(B, S, Dm)),
            "w_gate": _w((lambda *s: _rng.normal(s) * 0.1)(Dm, Df) * (Dm ** -0.5)),
            "w_up": _w((lambda *s: _rng.normal(s) * 0.1)(Dm, Df) * (Dm ** -0.5)),
            "w_down": _w((lambda *s: _rng.normal(s) * 0.1)(Df, Dm) * (Df ** -0.5)),
        }
    _B_in = _B_setup()

    return {
        "A_x": _A_in["x"],
        "A_wqkv": _A_in["wqkv"],
        "A_wo": _A_in["wo"],
        "B_x": _B_in["x"],
        "B_w_gate": _B_in["w_gate"],
        "B_w_up": _B_in["w_up"],
        "B_w_down": _B_in["w_down"],
    }

def reference(A_x, A_wqkv, A_wo, B_x, B_w_gate, B_w_up, B_w_down):
    def _A_ref(x, wqkv, wo):
        B, S, D = x.shape
        H = 32; Dh = D // H
        W, dil = 8, 2
        qkv = (lambda x, *d: x.transpose(*d))((x @ wqkv).reshape(B, S, 3, H, Dh), 2, 0, 3, 1, 4)
        q, k, v = qkv[0], qkv[1], qkv[2]
        scale = Dh ** -0.5
        pos = jnp.arange(S)
        off = jnp.arange(W) * dil
        idx = pos[:, None] - off[None, :]
        mask = idx >= 0
        idx_c = jnp.where(mask, idx, 0).reshape(-1)
        kg = k[:, :, idx_c, :].reshape(B, H, S, W, Dh)
        vg = v[:, :, idx_c, :].reshape(B, H, S, W, Dh)
        logits = jnp.einsum("bhsd,bhswd->bhsw", q, kg) * scale
        logits = jnp.where(mask[None, None, :, :], logits, -1e9)
        attn = _softmax(logits, axis=-1)
        o = jnp.einsum("bhsw,bhswd->bhsd", attn, vg)
        return (lambda x, *d: x.transpose(*d))(o, 0, 2, 1, 3).reshape(B, S, D) @ wo

    def _B_ref(x, w_gate, w_up, w_down):
        g = jnp.einsum("bsd,df->bsf", x, w_gate)
        u = jnp.einsum("bsd,df->bsf", x, w_up)
        h = _gelu(g) * u
        return jnp.einsum("bsf,fd->bsd", h, w_down)

    x = A_x
    xn = _layernorm(x, axis=-1)
    return x + _A_ref(xn, A_wqkv, A_wo) + _B_ref(xn, B_w_gate, B_w_up, B_w_down)
```

```python
import functools

import jax
import jax.numpy as jnp
from jax import lax
import jax.experimental.pallas as pl
import jax.experimental.pallas.tpu as pltpu

S = 2048
D = 512
F = 1376
W = 8
DIL = 2
PAD = 16
T = 512
NT = S // T
R = 8
FC = 256
SUB1 = 256
PIPE = 2

_NT_DIMS = (((1,), (1,)), ((), ()))
_LOG2E = 1.4426950408889634
_GC = 0.7978845608028654


def _gelu(x):
    inner = _GC * (x + 0.044715 * (x * x * x))
    return 0.5 * x * (1.0 + jnp.tanh(inner))


def _pack(x):
    return pltpu.bitcast(x.astype(jnp.bfloat16), jnp.int32)


def _bf(x):
    return pltpu.bitcast(x, jnp.bfloat16)


def _half(r):
    return r // 2 if isinstance(r, int) else pl.multiple_of(r // 2, 128)


def _kernel(x_hbm, wqkv_hbm, wo_hbm, wg_hbm, wu_hbm, wd_hbm, out_ref,
            wqkv_v, wo_v, wg_v, wu_v, wd_v, wqkv_p, wo_p, wo32,
            x_s, q_s, k_s, v_s, xn_s, xn_t, h_s, o_s, o_t, sems, xsems, wsems):
    i = pl.program_id(0)

    pairs = [(wo_hbm, wo_v), (wg_hbm, wg_v), (wu_hbm, wu_v), (wd_hbm, wd_v)]

    def copy(n):
        return pltpu.make_async_copy(pairs[n][0], pairs[n][1], sems.at[n])

    def xcopy(n):
        rows = pl.ds(n * T, T)
        return pltpu.make_async_copy(x_hbm.at[rows], x_s.at[rows], xsems.at[n])

    def wcopy(n):
        cols = pl.ds(n * D, D)
        return pltpu.make_async_copy(wqkv_hbm.at[:, cols], wqkv_v.at[:, cols],
                                     wsems.at[n])

    def layernorm(r0, dst, d0):
        for sb in range(T // 128):
            x = x_s[pl.ds(r0 + sb * 128, 128), :].astype(jnp.float32)
            m = jnp.mean(x, axis=-1, keepdims=True)
            xc = x - m
            var = jnp.mean(xc * xc, axis=-1, keepdims=True)
            xn = xc * lax.rsqrt(var + 1e-5)
            dst[pl.ds(d0 + sb * 64, 64), :] = _pack(xn)

    def perm_wqkv(m):
        RW = 128
        lane = lax.broadcasted_iota(jnp.int32, (RW // 2, 128), 1)
        grp = (lane % 32) // 8
        for j in range(4):
            idx = (lane % 8) * 16 + 4 * j + lane // 32
            for n in range(D // RW):
                res = None
                for s in range(4):
                    c0 = m * D + s * 128
                    src = pltpu.bitcast(
                        wqkv_v[n * RW:(n + 1) * RW, c0:c0 + 128], jnp.int32)
                    g = jnp.take_along_axis(src, idx, axis=1)
                    res = g if res is None else jnp.where(grp == s, g, res)
                c1 = m * D + j * 128
                wqkv_p[n * RW // 2:(n + 1) * RW // 2, c1:c1 + 128] = res

    def perm_wo(n):
        cols = slice(n * 128, (n + 1) * 128)
        for h in range(32):
            wo32[n, h * 17:h * 17 + 16, :] = wo_v[h * 16:(h + 1) * 16, cols].astype(
                jnp.float32)
        for j in range(4):
            for c in range(4):
                r1 = (j * 128 + c * 32) // 2
                wo_p[r1:r1 + 16, cols] = _pack(
                    wo32[n, pl.ds(4 * j + c, 32, stride=17), :])

    def attention(t0, dst):
        def stage1(c):
            r = c * R
            q = [q_s[j, pl.ds(t0 + r, R), :] for j in range(4)]
            accs = []
            for w in range(W):
                ks = PAD + r - DIL * w
                p = [q[j] * k_s[j, pl.ds(t0 + ks, R), :] for j in range(4)]
                accs.append((p[0] + p[1]) + (p[2] + p[3]))
            return [a + pltpu.roll(a, 64, 1) for a in accs]

        def stage2(c, accs):
            r = c * R
            logits = []
            for w, a in enumerate(accs):
                a = a + pltpu.roll(a, 32, 1)
                if w > 0 and r < DIL * w:
                    row = lax.broadcasted_iota(jnp.int32, (R, 128), 0) + (t0 + r)
                    a = jnp.where(row >= DIL * w, a, -1e9 * _LOG2E)
                logits.append(a)
            return logits

        def stage3(c, logits):
            r = c * R
            mx = functools.reduce(jnp.maximum, logits)
            ps = [jnp.exp2(l - mx) for l in logits]
            den = functools.reduce(lambda a, b: a + b, ps)
            inv = 1.0 / den
            for j in range(4):
                o = [ps[w] * v_s[j, pl.ds(t0 + PAD + r - DIL * w, R), :]
                     for w in range(W)]
                o = ((o[0] + o[1]) + (o[2] + o[3])) + ((o[4] + o[5]) + (o[6] + o[7]))
                dst[r // 2:(r + R) // 2, j * 128:(j + 1) * 128] = _pack(o * inv)

        n = T // R
        s1 = {}
        s2 = {}
        for c in range(n + PIPE):
            if c < n:
                s1[c] = stage1(c)
            c2 = c - PIPE // 2
            if 0 <= c2 < n:
                s2[c2] = stage2(c2, s1.pop(c2))
            c3 = c - PIPE
            if 0 <= c3 < n:
                stage3(c3, s2.pop(c3))

    def qkv(t0, which=(0, 1, 2), hooks=()):
        hooks = list(hooks)
        for sb in range(T // SUB1):
            r0 = t0 + sb * SUB1
            xn = _bf(xn_s[pl.ds(_half(r0), SUB1 // 2), :])
            for m_ in which:
                dst, off = ((q_s, 0), (k_s, PAD), (v_s, PAD))[m_]
                y = jnp.dot(xn, _bf(wqkv_p[:, m_ * D:(m_ + 1) * D]),
                            preferred_element_type=jnp.float32)
                if m_ == 0:
                    y = y * (0.25 * _LOG2E)
                for j in range(4):
                    dst[j, pl.ds(r0 + off, SUB1), :] = y[:, j * 128:(j + 1) * 128]
                if hooks:
                    hooks.pop(0)()

    @pl.when(i == 0)
    def _prologue():
        xcopy(0).start()
        wcopy(0).start()
        zeros = jnp.zeros((PAD, 128), jnp.float32)
        for j in range(4):
            k_s[j, 0:PAD, :] = zeros
            v_s[j, 0:PAD, :] = zeros
        xcopy(0).wait()
        layernorm(0, xn_s, 0)
        wcopy(0).wait()
        wcopy(1).start()
        perm_wqkv(0)
        wcopy(1).wait()
        wcopy(2).start()
        xcopy(1).start()
        qkv(0, (0,))
        perm_wqkv(1)
        wcopy(2).wait()
        for m in range(2, NT):
            xcopy(m).start()
        copy(0).start()
        qkv(0, (1,))
        perm_wqkv(2)
        xcopy(1).wait()
        qkv(0, (2,))
        layernorm(T, xn_s, T // 2)

    @pl.when(i == 1)
    def _phase1():
        for m in range(1, 4):
            copy(m).start()
        copy(0).wait()
        for m in range(2, NT):
            xcopy(m).wait()
        for m in range(1, NT):
            if m + 1 < NT:
                layernorm((m + 1) * T, xn_s, (m + 1) * T // 2)
            hooks = [functools.partial(perm_wo, n) for n in range(4)] if m == 1 else []
            qkv(m * T, hooks=hooks)
        attention(0, o_s)
        for n in range(1, 4):
            copy(n).wait()

    @pl.when(i >= 2)
    def _phase2():
        t0 = pl.multiple_of((i - 2) * T, T)
        t1 = pl.multiple_of(jnp.minimum(i - 1, NT - 1) * T, T)
        xn = _bf(xn_s[pl.ds(_half(t0), T // 2), :])
        for c in range(-(-F // FC)):
            c0 = c * FC
            c1 = min(c0 + FC, F)
            g = lax.dot_general(xn, wg_v[c0:c1, :], _NT_DIMS,
                                preferred_element_type=jnp.float32)
            u = lax.dot_general(xn, wu_v[c0:c1, :], _NT_DIMS,
                                preferred_element_type=jnp.float32)
            h_s[:, c0:c1] = _pack(_gelu(g) * u)
        acc = jnp.dot(_bf(h_s[...]), wd_v[...], preferred_element_type=jnp.float32)
        acc = acc + jnp.dot(_bf(o_s[...]), _bf(wo_p[...]), preferred_element_type=jnp.float32)
        out_ref[...] = (acc + x_s[pl.ds(t0, T), :].astype(jnp.float32)).astype(
            out_ref.dtype)
        attention(t1, o_t)
        o_s[...] = o_t[...]


@jax.jit
def pallas_parallel_sum__sliding_local_dilated__glu_gated_geglu__prompt_kernel(
    A_x: jax.Array,
    A_wqkv: jax.Array,
    A_wo: jax.Array,
    B_x: jax.Array,
    B_w_gate: jax.Array,
    B_w_up: jax.Array,
    B_w_down: jax.Array,
):
    x = A_x.reshape(S, D)
    hbm = pl.BlockSpec(memory_space=pltpu.HBM)
    bf = jnp.bfloat16
    f32 = jnp.float32
    i32 = jnp.int32
    out = pl.pallas_call(
        _kernel,
        grid=(2 + NT,),
        in_specs=[hbm] * 6,
        out_specs=pl.BlockSpec((T, D), lambda i: (jnp.maximum(i - 2, 0), 0)),
        out_shape=jax.ShapeDtypeStruct((S, D), A_x.dtype),
        scratch_shapes=[
            pltpu.VMEM((D, 3 * D), bf), pltpu.VMEM((D, D), bf),
            pltpu.VMEM((F, D), bf), pltpu.VMEM((F, D), bf), pltpu.VMEM((F, D), bf),
            pltpu.VMEM((D // 2, 3 * D), i32), pltpu.VMEM((D // 2, D), i32),
            pltpu.VMEM((4, 32 * 17, 128), f32),
            pltpu.VMEM((S, D), bf),
            pltpu.VMEM((4, S, 128), f32), pltpu.VMEM((4, S + PAD, 128), f32),
            pltpu.VMEM((4, S + PAD, 128), f32),
            pltpu.VMEM((S // 2, D), i32), pltpu.VMEM((T // 2, D), i32),
            pltpu.VMEM((T // 2, F), i32),
            pltpu.VMEM((T // 2, D), i32), pltpu.VMEM((T // 2, D), i32),
            pltpu.SemaphoreType.DMA((4,)), pltpu.SemaphoreType.DMA((NT,)),
            pltpu.SemaphoreType.DMA((3,)),
        ],
        compiler_params=pltpu.CompilerParams(
            dimension_semantics=("arbitrary",),
            vmem_limit_bytes=64 * 1024 * 1024,
        ),
    )(x, A_wqkv, A_wo, B_w_gate.T, B_w_up.T, B_w_down)
    return out.reshape(A_x.shape)
```

```python
import functools

import jax
import jax.numpy as jnp
from jax import lax
import jax.experimental.pallas as pl
import jax.experimental.pallas.tpu as pltpu

S = 2048
D = 512
F = 1376
W = 8
DIL = 2
PAD = 16
T = 512
NT = S // T
OSPLIT = (1, 4)
R = 8
FC = 256
SUB1 = 256
PIPE = 2

_NT_DIMS = (((1,), (1,)), ((), ()))
_LOG2E = 1.4426950408889634
_GC = 0.7978845608028654


def _gelu(x):
    inner = _GC * (x + 0.044715 * (x * x * x))
    return 0.5 * x * (1.0 + jnp.tanh(inner))


def _pack(x):
    return pltpu.bitcast(x.astype(jnp.bfloat16), jnp.int32)


def _bf(x):
    return pltpu.bitcast(x, jnp.bfloat16)


def _half(r):
    return r // 2 if isinstance(r, int) else pl.multiple_of(r // 2, 128)


def _kernel(x_hbm, wqkv_hbm, wo_hbm, wg_hbm, wu_hbm, wd_hbm, out_hbm,
            wqkv_v, wo_v, wg_v, wu_v, wd_v, wqkv_p, wo_p, wo32,
            x_s, q_s, k_s, v_s, xn_s, xn_t, h_s, o_s, o_t, out_s, sems, xsems, wsems,
            osems):
    i = pl.program_id(0)

    pairs = [(wo_hbm, wo_v), (wg_hbm, wg_v), (wu_hbm, wu_v), (wd_hbm, wd_v)]

    def copy(n):
        return pltpu.make_async_copy(pairs[n][0], pairs[n][1], sems.at[n])

    def xcopy(n):
        rows = pl.ds(n * T, T)
        return pltpu.make_async_copy(x_hbm.at[rows], x_s.at[rows], xsems.at[n])

    def wcopy(n):
        cols = pl.ds(n * D, D)
        return pltpu.make_async_copy(wqkv_hbm.at[:, cols], wqkv_v.at[:, cols],
                                     wsems.at[n])

    def layernorm(r0, dst, d0, subs=None):
        for sb in (range(T // 128) if subs is None else subs):
            x = x_s[pl.ds(r0 + sb * 128, 128), :].astype(jnp.float32)
            m = jnp.mean(x, axis=-1, keepdims=True)
            xc = x - m
            var = jnp.mean(xc * xc, axis=-1, keepdims=True)
            xn = xc * lax.rsqrt(var + 1e-5)
            dst[pl.ds(d0 + sb * 64, 64), :] = _pack(xn)

    def perm_wqkv(m):
        RW = 128
        lane = lax.broadcasted_iota(jnp.int32, (RW // 2, 128), 1)
        grp = (lane % 32) // 8
        for j in range(4):
            idx = (lane % 8) * 16 + 4 * j + lane // 32
            for n in range(D // RW):
                res = None
                for s in range(4):
                    c0 = m * D + s * 128
                    src = pltpu.bitcast(
                        wqkv_v[n * RW:(n + 1) * RW, c0:c0 + 128], jnp.int32)
                    g = jnp.take_along_axis(src, idx, axis=1)
                    res = g if res is None else jnp.where(grp == s, g, res)
                c1 = m * D + j * 128
                wqkv_p[n * RW // 2:(n + 1) * RW // 2, c1:c1 + 128] = res

    def perm_wo(n):
        cols = slice(n * 128, (n + 1) * 128)
        for h in range(32):
            wo32[n, h * 17:h * 17 + 16, :] = wo_v[h * 16:(h + 1) * 16, cols].astype(
                jnp.float32)
        for j in range(4):
            for c in range(4):
                r1 = (j * 128 + c * 32) // 2
                wo_p[r1:r1 + 16, cols] = _pack(
                    wo32[n, pl.ds(4 * j + c, 32, stride=17), :])

    def attention(t0, dst):
        def stage1(c):
            r = c * R
            q = [q_s[j, pl.ds(t0 + r, R), :] for j in range(4)]
            accs = []
            for w in range(W):
                ks = PAD + r - DIL * w
                p = [q[j] * k_s[j, pl.ds(t0 + ks, R), :] for j in range(4)]
                accs.append((p[0] + p[1]) + (p[2] + p[3]))
            return [a + pltpu.roll(a, 64, 1) for a in accs]

        def stage2(c, accs):
            r = c * R
            logits = []
            for w, a in enumerate(accs):
                a = a + pltpu.roll(a, 32, 1)
                if w > 0 and r < DIL * w:
                    row = lax.broadcasted_iota(jnp.int32, (R, 128), 0) + (t0 + r)
                    a = jnp.where(row >= DIL * w, a, -1e9 * _LOG2E)
                logits.append(a)
            return logits

        def stage3(c, logits):
            r = c * R
            mx = functools.reduce(jnp.maximum, logits)
            ps = [jnp.exp2(l - mx) for l in logits]
            den = functools.reduce(lambda a, b: a + b, ps)
            inv = pl.reciprocal(den, approx=True)
            inv = inv * (2.0 - den * inv)
            for j in range(4):
                o = [ps[w] * v_s[j, pl.ds(t0 + PAD + r - DIL * w, R), :]
                     for w in range(W)]
                o = ((o[0] + o[1]) + (o[2] + o[3])) + ((o[4] + o[5]) + (o[6] + o[7]))
                dst[r // 2:(r + R) // 2, j * 128:(j + 1) * 128] = _pack(o * inv)

        n = T // R
        s1 = {}
        s2 = {}
        for c in range(n + PIPE):
            if c < n:
                s1[c] = stage1(c)
            c2 = c - PIPE // 2
            if 0 <= c2 < n:
                s2[c2] = stage2(c2, s1.pop(c2))
            c3 = c - PIPE
            if 0 <= c3 < n:
                stage3(c3, s2.pop(c3))

    def qkv(t0, which=(0, 1, 2), hooks=()):
        hooks = list(hooks)
        for sb in range(T // SUB1):
            r0 = t0 + sb * SUB1
            xn = _bf(xn_s[pl.ds(_half(r0), SUB1 // 2), :])
            for m_ in which:
                dst, off = ((q_s, 0), (k_s, PAD), (v_s, PAD))[m_]
                y = jnp.dot(xn, _bf(wqkv_p[:, m_ * D:(m_ + 1) * D]),
                            preferred_element_type=jnp.float32)
                if m_ == 0:
                    y = y * (0.25 * _LOG2E)
                for j in range(4):
                    dst[j, pl.ds(r0 + off, SUB1), :] = y[:, j * 128:(j + 1) * 128]
                if hooks:
                    hooks.pop(0)()

    @pl.when(i == 0)
    def _prologue():
        wcopy(0).start()
        xcopy(0).start()
        wcopy(1).start()
        zeros = jnp.zeros((PAD, 128), jnp.float32)
        for j in range(4):
            k_s[j, 0:PAD, :] = zeros
            v_s[j, 0:PAD, :] = zeros
        wcopy(0).wait()
        wcopy(2).start()
        perm_wqkv(0)
        xcopy(0).wait()
        layernorm(0, xn_s, 0, (0, 1))
        wcopy(1).wait()
        xcopy(1).start()
        layernorm(0, xn_s, 0, (2, 3))
        qkv(0, (0,))
        perm_wqkv(1)
        wcopy(2).wait()
        xcopy(1).wait()
        for m in range(2, NT):
            xcopy(m).start()
        for m in range(4):
            copy(m).start()
        qkv(0, (1,))
        perm_wqkv(2)
        qkv(0, (2,))
        layernorm(T, xn_s, T // 2)
        qkv(T, (0,))
        for m in range(2, NT):
            xcopy(m).wait()
        qkv(T, (1, 2))
        for m in range(2, NT):
            layernorm(m * T, xn_s, m * T // 2)
            qkv(m * T)
        attention(0, o_s)
        for n in range(4):
            copy(n).wait()

    def ocopy(r0, n, p, nr):
        rows = pl.ds(r0, nr)
        return pltpu.make_async_copy(out_s.at[rows], out_hbm.at[rows], osems.at[n, p])

    @pl.when(i >= 1)
    def _phase2():
        for n in range(4):
            perm_wo(n)
        for half, (o_rd, o_wr) in enumerate(((o_s, o_t), (o_t, o_s))):
            n = (i - 1) * 2 + half
            t0 = pl.multiple_of(n * T, T)
            t1 = pl.multiple_of(jnp.minimum(n + 1, NT - 1) * T, T)
            xn = _bf(xn_s[pl.ds(_half(t0), T // 2), :])
            for c in range(-(-F // FC)):
                c0 = c * FC
                c1 = min(c0 + FC, F)
                g = lax.dot_general(xn, wg_v[c0:c1, :], _NT_DIMS,
                                    preferred_element_type=jnp.float32)
                u = lax.dot_general(xn, wu_v[c0:c1, :], _NT_DIMS,
                                    preferred_element_type=jnp.float32)
                h_s[:, c0:c1] = _pack(_gelu(g) * u)
            parts = OSPLIT[half]
            nr = T // parts
            for p in range(parts):
                rs = slice(p * nr // 2, (p + 1) * nr // 2)
                r0 = pl.multiple_of(t0 + p * nr, nr)
                acc = jnp.dot(_bf(h_s[rs, :]), wd_v[...],
                              preferred_element_type=jnp.float32)
                acc = acc + jnp.dot(_bf(o_rd[rs, :]), _bf(wo_p[...]),
                                    preferred_element_type=jnp.float32)
                out_s[pl.ds(r0, nr), :] = (
                    acc + x_s[pl.ds(r0, nr), :].astype(jnp.float32)).astype(out_s.dtype)
                ocopy(r0, n, p, nr).start()
            attention(t1, o_wr)

    @pl.when(i == NT // 2)
    def _drain():
        for n in range(NT):
            parts = OSPLIT[n % 2]
            for p in range(parts):
                ocopy(n * T + p * (T // parts), n, p, T // parts).wait()


@jax.jit
def pallas_parallel_sum__sliding_local_dilated__glu_gated_geglu__prompt_kernel(
    A_x: jax.Array,
    A_wqkv: jax.Array,
    A_wo: jax.Array,
    B_x: jax.Array,
    B_w_gate: jax.Array,
    B_w_up: jax.Array,
    B_w_down: jax.Array,
):
    x = A_x.reshape(S, D)
    hbm = pl.BlockSpec(memory_space=pltpu.HBM)
    bf = jnp.bfloat16
    f32 = jnp.float32
    i32 = jnp.int32
    out = pl.pallas_call(
        _kernel,
        grid=(1 + NT // 2,),
        in_specs=[hbm] * 6,
        out_specs=hbm,
        out_shape=jax.ShapeDtypeStruct((S, D), A_x.dtype),
        scratch_shapes=[
            pltpu.VMEM((D, 3 * D), bf), pltpu.VMEM((D, D), bf),
            pltpu.VMEM((F, D), bf), pltpu.VMEM((F, D), bf), pltpu.VMEM((F, D), bf),
            pltpu.VMEM((D // 2, 3 * D), i32), pltpu.VMEM((D // 2, D), i32),
            pltpu.VMEM((4, 32 * 17, 128), f32),
            pltpu.VMEM((S, D), bf),
            pltpu.VMEM((4, S, 128), f32), pltpu.VMEM((4, S + PAD, 128), f32),
            pltpu.VMEM((4, S + PAD, 128), f32),
            pltpu.VMEM((S // 2, D), i32), pltpu.VMEM((T // 2, D), i32),
            pltpu.VMEM((T // 2, F), i32),
            pltpu.VMEM((T // 2, D), i32), pltpu.VMEM((T // 2, D), i32),
            pltpu.VMEM((S, D), bf),
            pltpu.SemaphoreType.DMA((4,)), pltpu.SemaphoreType.DMA((NT,)),
            pltpu.SemaphoreType.DMA((3,)), pltpu.SemaphoreType.DMA((NT, 4)),
        ],
        compiler_params=pltpu.CompilerParams(
            dimension_semantics=("arbitrary",),
            vmem_limit_bytes=64 * 1024 * 1024,
            flags={'XLA_TPU_EVENLY_DISTRIBUTE_CRITICAL_NODES': True},
        ),
    )(x, A_wqkv, A_wo, B_w_gate.T, B_w_up.T, B_w_down)
    return out.reshape(A_x.shape)
```

```python
import functools

import jax
import jax.numpy as jnp
from jax import lax
import jax.experimental.pallas as pl
import jax.experimental.pallas.tpu as pltpu

S = 2048
D = 512
F = 1376
W = 8
DIL = 2
PAD = 16
T = 512
NT = S // T
OSPLIT = (1, 4)
PRW = 64
R = 8
FC = 256
SUB1 = 256
PIPE = 2

_NT_DIMS = (((1,), (1,)), ((), ()))
_LOG2E = 1.4426950408889634
_GC = 0.7978845608028654


def _gelu(x):
    inner = _GC * (x + 0.044715 * (x * x * x))
    return 0.5 * x * (1.0 + jnp.tanh(inner))


def _pack(x):
    return pltpu.bitcast(x.astype(jnp.bfloat16), jnp.int32)


def _bf(x):
    return pltpu.bitcast(x, jnp.bfloat16)


def _hslot(h):
    return (h % 8) * 4 + h // 8


def _half(r):
    return r // 2 if isinstance(r, int) else pl.multiple_of(r // 2, 128)


def _kernel(x_hbm, wqkv_hbm, wo_hbm, wg_hbm, wu_hbm, wd_hbm, out_hbm,
            wqkv_v, wo_v, wg_v, wu_v, wd_v, wqkv_p, wo_p, wo32,
            x_s, q_s, k_s, v_s, xn_s, h_s, o_s, o_t, out_s, sems, xsems, wsems,
            osems):
    i = pl.program_id(0)

    pairs = [(wo_hbm, wo_v), (wg_hbm, wg_v), (wu_hbm, wu_v), (wd_hbm, wd_v)]

    def copy(n):
        return pltpu.make_async_copy(pairs[n][0], pairs[n][1], sems.at[n])

    def xcopy(n):
        rows = pl.ds(n * T, T)
        return pltpu.make_async_copy(x_hbm.at[rows], x_s.at[rows], xsems.at[n])

    def wcopy(n):
        cols = pl.ds(n * D, D)
        return pltpu.make_async_copy(wqkv_hbm.at[:, cols], wqkv_v.at[:, cols],
                                     wsems.at[n])

    def layernorm(r0, dst, d0, subs=None):
        for sb in (range(T // 128) if subs is None else subs):
            x = x_s[pl.ds(r0 + sb * 128, 128), :].astype(jnp.float32)
            m = jnp.mean(x, axis=-1, keepdims=True)
            xc = x - m
            var = jnp.mean(xc * xc, axis=-1, keepdims=True)
            xn = xc * lax.rsqrt(var + 1e-5)
            dst[pl.ds(d0 + sb * 64, 64), :] = _pack(xn)

    def perm_wqkv(m):
        RW = PRW
        lane = lax.broadcasted_iota(jnp.int32, (RW // 2, 128), 1)
        idx = (lane % 32) * 4 + lane // 32

        def swap(r, bit, sh):
            hi = (lane & sh) != 0
            nxt = list(r)
            for a in range(4):
                if a & bit == 0:
                    b = a | bit
                    nxt[a] = jnp.where(hi, pltpu.roll(r[b], sh, 1), r[a])
                    nxt[b] = jnp.where(hi, r[b], pltpu.roll(r[a], 128 - sh, 1))
            return nxt

        nb = D // RW
        st = {}
        for t in range(nb + 2):
            if t < nb:
                st[t] = swap([pltpu.bitcast(
                    wqkv_v[t * RW:(t + 1) * RW, m * D + s * 128:m * D + (s + 1) * 128],
                    jnp.int32) for s in range(4)], 1, 4)
            if 0 <= t - 1 < nb:
                st[t - 1] = swap(st[t - 1], 2, 8)
            if 0 <= t - 2 < nb:
                n = t - 2
                r = st.pop(n)
                for j in range(4):
                    c1 = m * D + j * 128
                    wqkv_p[n * RW // 2:(n + 1) * RW // 2, c1:c1 + 128] = (
                        jnp.take_along_axis(r[j], idx, axis=1))

    def perm_wo(n):
        cols = slice(n * 128, (n + 1) * 128)
        for h in range(32):
            wo32[n, _hslot(h) * 17:_hslot(h) * 17 + 16, :] = wo_v[h * 16:(h + 1) * 16, cols].astype(
                jnp.float32)
        for j in range(4):
            for c in range(4):
                r1 = (j * 128 + c * 32) // 2
                wo_p[r1:r1 + 16, cols] = _pack(
                    wo32[n, pl.ds(4 * j + c, 32, stride=17), :])

    def attention(t0, dst):
        def stage1(c):
            r = c * R
            q = [q_s[j, pl.ds(t0 + r, R), :] for j in range(4)]
            accs = []
            for w in range(W):
                ks = PAD + r - DIL * w
                p = [q[j] * k_s[j, pl.ds(t0 + ks, R), :] for j in range(4)]
                accs.append((p[0] + p[1]) + (p[2] + p[3]))
            return [a + pltpu.roll(a, 64, 1) for a in accs]

        def stage2(c, accs):
            r = c * R
            logits = []
            for w, a in enumerate(accs):
                a = a + pltpu.roll(a, 32, 1)
                if w > 0 and r < DIL * w:
                    row = lax.broadcasted_iota(jnp.int32, (R, 128), 0) + (t0 + r)
                    a = jnp.where(row >= DIL * w, a, -1e9 * _LOG2E)
                logits.append(a)
            return logits

        def stage3(c, logits):
            r = c * R
            mx = functools.reduce(jnp.maximum, logits)
            ps = [jnp.exp2(l - mx) for l in logits]
            den = functools.reduce(lambda a, b: a + b, ps)
            inv = pl.reciprocal(den, approx=True)
            inv = inv * (2.0 - den * inv)
            for j in range(4):
                o = [ps[w] * v_s[j, pl.ds(t0 + PAD + r - DIL * w, R), :]
                     for w in range(W)]
                o = ((o[0] + o[1]) + (o[2] + o[3])) + ((o[4] + o[5]) + (o[6] + o[7]))
                dst[r // 2:(r + R) // 2, j * 128:(j + 1) * 128] = _pack(o * inv)

        n = T // R
        s1 = {}
        s2 = {}
        for c in range(n + PIPE):
            if c < n:
                s1[c] = stage1(c)
            c2 = c - PIPE // 2
            if 0 <= c2 < n:
                s2[c2] = stage2(c2, s1.pop(c2))
            c3 = c - PIPE
            if 0 <= c3 < n:
                stage3(c3, s2.pop(c3))

    def qkv(t0, which=(0, 1, 2), hooks=()):
        hooks = list(hooks)
        for sb in range(T // SUB1):
            r0 = t0 + sb * SUB1
            xn = _bf(xn_s[pl.ds(_half(r0), SUB1 // 2), :])
            for m_ in which:
                dst, off = ((q_s, 0), (k_s, PAD), (v_s, PAD))[m_]
                y = jnp.dot(xn, _bf(wqkv_p[:, m_ * D:(m_ + 1) * D]),
                            preferred_element_type=jnp.float32)
                if m_ == 0:
                    y = y * (0.25 * _LOG2E)
                for j in range(4):
                    dst[j, pl.ds(r0 + off, SUB1), :] = y[:, j * 128:(j + 1) * 128]
                if hooks:
                    hooks.pop(0)()

    @pl.when(i == 0)
    def _prologue():
        wcopy(0).start()
        xcopy(0).start()
        wcopy(1).start()
        zeros = jnp.zeros((PAD, 128), jnp.float32)
        for j in range(4):
            k_s[j, 0:PAD, :] = zeros
            v_s[j, 0:PAD, :] = zeros
        wcopy(0).wait()
        wcopy(2).start()
        perm_wqkv(0)
        xcopy(0).wait()
        layernorm(0, xn_s, 0, (0, 1))
        wcopy(1).wait()
        xcopy(1).start()
        layernorm(0, xn_s, 0, (2, 3))
        qkv(0, (0,))
        perm_wqkv(1)
        wcopy(2).wait()
        xcopy(1).wait()
        for m in range(2, NT):
            xcopy(m).start()
        for m in range(4):
            copy(m).start()
        qkv(0, (1,))
        perm_wqkv(2)
        qkv(0, (2,))
        layernorm(T, xn_s, T // 2)
        qkv(T, (0,))
        for m in range(2, NT):
            xcopy(m).wait()
        qkv(T, (1, 2))
        for m in range(2, NT):
            layernorm(m * T, xn_s, m * T // 2)
            qkv(m * T)
        attention(0, o_s)
        for n in range(4):
            copy(n).wait()

    def ocopy(r0, n, p, nr):
        rows = pl.ds(r0, nr)
        return pltpu.make_async_copy(out_s.at[rows], out_hbm.at[rows], osems.at[n, p])

    @pl.when(i >= 1)
    def _phase2():
        for n in range(4):
            perm_wo(n)
        for half, (o_rd, o_wr) in enumerate(((o_s, o_t), (o_t, o_s))):
            n = (i - 1) * 2 + half
            t0 = pl.multiple_of(n * T, T)
            t1 = pl.multiple_of(jnp.minimum(n + 1, NT - 1) * T, T)
            xn = _bf(xn_s[pl.ds(_half(t0), T // 2), :])
            for c in range(-(-F // FC)):
                c0 = c * FC
                c1 = min(c0 + FC, F)
                g = lax.dot_general(xn, wg_v[c0:c1, :], _NT_DIMS,
                                    preferred_element_type=jnp.float32)
                u = lax.dot_general(xn, wu_v[c0:c1, :], _NT_DIMS,
                                    preferred_element_type=jnp.float32)
                h_s[:, c0:c1] = _pack(_gelu(g) * u)
            parts = OSPLIT[half]
            nr = T // parts
            for p in range(parts):
                rs = slice(p * nr // 2, (p + 1) * nr // 2)
                r0 = pl.multiple_of(t0 + p * nr, nr)
                acc = jnp.dot(_bf(h_s[rs, :]), wd_v[...],
                              preferred_element_type=jnp.float32)
                acc = acc + jnp.dot(_bf(o_rd[rs, :]), _bf(wo_p[...]),
                                    preferred_element_type=jnp.float32)
                out_s[pl.ds(r0, nr), :] = (
                    acc + x_s[pl.ds(r0, nr), :].astype(jnp.float32)).astype(out_s.dtype)
                ocopy(r0, n, p, nr).start()
            attention(t1, o_wr)

    @pl.when(i == NT // 2)
    def _drain():
        for n in range(NT):
            parts = OSPLIT[n % 2]
            for p in range(parts):
                ocopy(n * T + p * (T // parts), n, p, T // parts).wait()


@jax.jit
def pallas_parallel_sum__sliding_local_dilated__glu_gated_geglu__prompt_kernel(
    A_x: jax.Array,
    A_wqkv: jax.Array,
    A_wo: jax.Array,
    B_x: jax.Array,
    B_w_gate: jax.Array,
    B_w_up: jax.Array,
    B_w_down: jax.Array,
):
    x = A_x.reshape(S, D)
    hbm = pl.BlockSpec(memory_space=pltpu.HBM)
    bf = jnp.bfloat16
    f32 = jnp.float32
    i32 = jnp.int32
    out = pl.pallas_call(
        _kernel,
        grid=(1 + NT // 2,),
        in_specs=[hbm] * 6,
        out_specs=hbm,
        out_shape=jax.ShapeDtypeStruct((S, D), A_x.dtype),
        scratch_shapes=[
            pltpu.VMEM((D, 3 * D), bf), pltpu.VMEM((D, D), bf),
            pltpu.VMEM((F, D), bf), pltpu.VMEM((F, D), bf), pltpu.VMEM((F, D), bf),
            pltpu.VMEM((D // 2, 3 * D), i32), pltpu.VMEM((D // 2, D), i32),
            pltpu.VMEM((4, 32 * 17, 128), f32),
            pltpu.VMEM((S, D), bf),
            pltpu.VMEM((4, S, 128), f32), pltpu.VMEM((4, S + PAD, 128), f32),
            pltpu.VMEM((4, S + PAD, 128), f32),
            pltpu.VMEM((S // 2, D), i32),
            pltpu.VMEM((T // 2, F), i32),
            pltpu.VMEM((T // 2, D), i32), pltpu.VMEM((T // 2, D), i32),
            pltpu.VMEM((S, D), bf),
            pltpu.SemaphoreType.DMA((4,)), pltpu.SemaphoreType.DMA((NT,)),
            pltpu.SemaphoreType.DMA((3,)), pltpu.SemaphoreType.DMA((NT, 4)),
        ],
        compiler_params=pltpu.CompilerParams(
            dimension_semantics=("arbitrary",),
            vmem_limit_bytes=64 * 1024 * 1024,
            flags={'XLA_TPU_EVENLY_DISTRIBUTE_CRITICAL_NODES': True},
        ),
    )(x, A_wqkv, A_wo, B_w_gate.T, B_w_up.T, B_w_down)
    return out.reshape(A_x.shape)
```
